```python
import os as _os
_os.environ.setdefault("JAX_PLATFORMS", "cpu")
import jax
import jax.numpy as jnp

def _softmax(x, axis=-1):
    return jax.nn.softmax(x, axis=axis)
def _gelu(x):
    return jax.nn.gelu(x, approximate=True)
def _silu(x):
    return jax.nn.silu(x)
def _sigmoid(x):
    return jax.nn.sigmoid(x)
def _layernorm(x, axis=-1, eps=1e-5):
    m = jnp.mean(x, axis=axis, keepdims=True)
    v = jnp.var(x, axis=axis, keepdims=True)
    return (x - m) / jnp.sqrt(v + eps)
def _scatter_add(tgt, idx, src, axis=0):
    return tgt.at[idx].add(src)
def _segment_sum(src, seg, n):
    return jax.ops.segment_sum(src, seg, n)
class _Rng:
    def __init__(self, key):
        self._k = key
    def _next(self):
        self._k, sub = jax.random.split(self._k)
        return sub
    def normal(self, shape):
        return jax.random.normal(self._next(), shape, dtype=jnp.bfloat16)
    def randint(self, lo, hi, shape):
        return jax.random.randint(self._next(), shape, lo, hi, dtype=jnp.int32)
    def uniform(self, shape, lo=0.0, hi=1.0):
        return jax.random.uniform(self._next(), shape, jnp.bfloat16, lo, hi)
    def permutation(self, n):
        return jax.random.permutation(self._next(), n)


kernel_name = 'parallel_sum__softmax_full_mha__glu_gated_swiglu__prompt'

def setup_inputs():
    _rng = _Rng(jax.random.key(int.from_bytes(__import__("os").urandom(4), "little")))
    _w = (lambda a: (lambda t: t.astype(jnp.bfloat16) if jnp.issubdtype(t.dtype, jnp.floating) else t)(jnp.asarray(a)))
    def _A_setup():
        B, S, D = 1, 2048, 448
        return {
            "x": _w((lambda *s: _rng.normal(s) * 0.05)(B, S, D)),
            "wqkv": _w((lambda *s: _rng.normal(s) * 0.05)(D, 3 * D)),
            "wo": _w((lambda *s: _rng.normal(s) * 0.05)(D, D)),
        }
    _A_in = _A_setup()

    def _B_setup():
        B, S, D, F = 1, 2048, 448, 1792
        return {
            "x": _w((lambda *s: _rng.normal(s) * 0.05)(B, S, D)),
            "w1": _w((lambda *s: _rng.normal(s) * 0.05)(D, F) * (2.0 / D) ** 0.5),
            "w3": _w((lambda *s: _rng.normal(s) * 0.05)(D, F) * (2.0 / D) ** 0.5),
            "w2": _w((lambda *s: _rng.normal(s) * 0.05)(F, D) * (2.0 / F) ** 0.5),
        }
    _B_in = _B_setup()

    return {
        "A_x": _A_in["x"],
        "A_wqkv": _A_in["wqkv"],
        "A_wo": _A_in["wo"],
        "B_x": _B_in["x"],
        "B_w1": _B_in["w1"],
        "B_w3": _B_in["w3"],
        "B_w2": _B_in["w2"],
    }

def reference(A_x, A_wqkv, A_wo, B_x, B_w1, B_w3, B_w2):
    def _A_ref(x, wqkv, wo):
        B, S, D = x.shape
        H = 16; Dh = D // H
        qkv = (lambda x, *d: x.transpose(*d))((x @ wqkv).reshape(B, S, 3, H, Dh), 2, 0, 3, 1, 4)
        q, k, v = qkv[0], qkv[1], qkv[2]
        scale = Dh ** -0.5
        scores = jnp.einsum("bhqd,bhkd->bhqk", q, k) * scale
        p = _softmax(scores, axis=-1)
        o = jnp.einsum("bhqk,bhkd->bhqd", p, v)
        return (lambda x, *d: x.transpose(*d))(o, 0, 2, 1, 3).reshape(B, S, D) @ wo

    def _B_ref(x, w1, w3, w2):
        gate = jnp.einsum("bsd,df->bsf", x, w1)
        up = jnp.einsum("bsd,df->bsf", x, w3)
        h = _silu(gate) * up
        out = jnp.einsum("bsf,fd->bsd", h, w2)
        return out

    x = A_x
    xn = _layernorm(x, axis=-1)
    return x + _A_ref(xn, A_wqkv, A_wo) + _B_ref(xn, B_w1, B_w3, B_w2)
```

```python
import functools
import math

import jax
import jax.numpy as jnp
from jax import lax
import jax.experimental.pallas as pl
import jax.experimental.pallas.tpu as pltpu

_BF = jnp.bfloat16
_F32 = jnp.float32
_U32 = jnp.uint32

S, D, F, H = 2048, 448, 1792, 16
DH = D // H
BQ = 512
HB = BQ // 2
NQ = S // BQ
GW = 4 * DH
FH = F // 2
EPS = 1e-5
QSCALE = DH ** -0.5 * math.log2(math.e)


def _bf(x):
    return pltpu.bitcast(x, _BF)


def _u32(x):
    return pltpu.bitcast(x, _U32)


def _pk(x):
    return _u32(x.astype(_BF))


def _dot(a, b):
    return jnp.dot(a, b, preferred_element_type=_F32)


def _dot_nt(a, b):
    return lax.dot_general(a, b, (((1,), (1,)), ((), ())), preferred_element_type=_F32)


def _cat(xs, axis):
    return jnp.concatenate(xs, axis=axis)


def _kernel(x_hbm, wqkv_hbm, wo_hbm, w1_hbm, w3_hbm, w2_hbm, out_hbm,
            x_v, wqkv_v, wo_v, w1_v, w3_v, w2_v,
            wt_s, wot_s, xt_s, xn_s, k_s, q_s, v_s, sa, sb, o_s, h_s, y_s, out_v, sems, *, CK, fsplit, ffn_at):
    x_cp = [pltpu.make_async_copy(x_hbm.at[:, pl.ds(c * BQ, BQ)], x_v.at[c], sems.at[c]) for c in range(NQ)]
    wqkv_cp = pltpu.make_async_copy(wqkv_hbm, wqkv_v, sems.at[4])
    wo_cp = pltpu.make_async_copy(wo_hbm, wo_v, sems.at[5])
    w_cp = [pltpu.make_async_copy(src.at[:, pl.ds(i * FH, FH)], dst.at[i], sems.at[6 + 3 * i + j])
            for i in range(2) for j, (src, dst) in enumerate(((w1_hbm, w1_v), (w3_hbm, w3_v), (w2_hbm, w2_v)))]

    def out_cp(qb):
        return pltpu.make_async_copy(out_v.at[qb], out_hbm.at[:, pl.ds(pl.multiple_of(qb * BQ, BQ), BQ)], sems.at[12 + qb])

    x_cp[0].start()
    wqkv_cp.start()
    sa[0:8, :] = jnp.zeros((8, BQ), _F32)
    sb[0:8, :] = jnp.zeros((8, BQ), _F32)
    h_s[0:8, :] = jnp.zeros((8, FH), _U32)
    o_s[...] = jnp.zeros(o_s.shape, _F32)
    y_s[...] = jnp.zeros(y_s.shape, _F32)
    x_cp[0].wait()
    for c in range(1, NQ):
        x_cp[c].start()
    wo_cp.start()

    row8 = lax.broadcasted_iota(jnp.int32, (8, BQ), 0)
    low4 = row8 < 4

    def layer_norm(c):
        def half(cols):
            x = x_v[c, :, cols].astype(_F32)
            mu = jnp.sum(x, axis=0, keepdims=True) * (1.0 / D)
            xc = x - mu
            var = jnp.sum(xc * xc, axis=0, keepdims=True) * (1.0 / D)
            return xc * lax.rsqrt(var + EPS)
        for t in range(HB // 128):
            cols = slice(t * 128, (t + 1) * 128)
            a = half(cols)
            b = half(slice(HB + t * 128, HB + (t + 1) * 128))
            zb = b[320:384].astype(_BF)
            za = a[384:448].astype(_BF)
            xt_s[c, 0:160, cols] = _pk(a[0:320])
            xt_s[c, 160:192, cols] = _pk(a[320:384] - zb.astype(_F32))
            xt_s[c, 192:352, cols] = _pk(b[0:320])
            xt_s[c, 352:384, cols] = _pk(b[384:448] - za.astype(_F32))
            xt_s[c, 384:416, cols] = _u32(zb)
            xt_s[c, 416:448, cols] = _u32(za)

    def proj(c, i):
        rows = slice(i * D // 2, (i + 1) * D // 2)
        xa, xb, xz = _bf(xt_s[c, 0:192]), _bf(xt_s[c, 192:384]), _bf(xt_s[c, 384:448])
        y = _dot(_bf(wt_s[rows, 0:256]), _cat([xa[0:256], xb[0:256]], 1))
        z = _dot(_bf(wt_s[rows, 512:640]), xz)
        ya = _dot(_bf(wt_s[rows, 256:384]), xa[256:384])
        yb = _dot(_bf(wt_s[rows, 384:512]), xb[256:384])
        return y + _cat([ya + z, yb + z], 1)

    def proj_k(c):
        kt = proj(c, 1)
        for g in range(4):
            kg = _cat([kt[g * GW:(g + 1) * GW], jnp.zeros((128 - GW, BQ), _F32)], 0)
            k_s[g, c * BQ // 2:(c + 1) * BQ // 2, :] = _u32(kg.astype(_BF).T)

    def proj_v(c):
        cols = slice(c * BQ, (c + 1) * BQ)
        vt = proj(c, 2)
        for p in range(H // 2):
            b = 2 * DH * p
            mid = vt[b + 24:b + 32]
            v_s[2 * p, :, cols] = _pk(_cat([vt[b:b + 24], jnp.where(low4, mid, 1.0)], 0))
            v_s[2 * p + 1, :, cols] = _pk(_cat([jnp.where(low4, 1.0, mid), vt[b + 32:b + 56]], 0))

    def proj_q(c):
        qt = _pk(proj(c, 0) * QSCALE)
        q_s[2 * c] = qt[0:D // 4]
        q_s[2 * c + 1] = qt[D // 4:D // 2]
        xn_s[c] = _u32(_bf(xt_s[c]).T)

    layer_norm(0)
    wqkv_cp.wait()
    for cp in w_cp:
        cp.start()
    w = wqkv_v[...]
    wt_s[...] = _u32(_cat([w[0:384], w[256:320], w[384:448], w[320:448]], 0).T)
    proj_k(0)
    proj_v(0)
    for c in range(1, NQ):
        x_cp[c].wait()
    wo_cp.wait()
    for c in range(1, NQ):
        layer_norm(c)
        proj_q(c - 1)
        proj_k(c)
        proj_v(c)
    for i in range(2):
        wo = _cat([wo_v[i * D // 2:(i + 1) * D // 2], jnp.zeros((256 - D // 2, D), _BF)], 0)
        wot_s[i] = _u32(wo.T)
    proj_q(NQ - 1)
    for cp in w_cp:
        cp.wait()

    NC = S // CK
    HH = H // 2

    def half_block(it):
        qb = it // 2
        hf = it % 2

        def q_head(h):
            g, j = divmod(h, 4)
            w = q_s[it, g * GW // 2:(g + 1) * GW // 2, :]
            r = lax.broadcasted_iota(jnp.int32, w.shape, 0)
            w = jnp.where((r >= DH // 2 * j) & (r < DH // 2 * (j + 1)), w, jnp.zeros_like(w))
            w = _cat([w, jnp.zeros(((128 - GW) // 2, BQ), _U32)], 0)
            return _bf(w)

        def qk(h, qm, c, mx):
            s_w = (sa, sb)[h % 2]
            s = _dot(_bf(k_s[2 * hf + h // 4, c * CK // 2:(c + 1) * CK // 2, :]), qm)
            s_w[c * CK:(c + 1) * CK, :] = s
            s8 = jnp.max(s.reshape(CK // 8, 8, BQ), axis=0)
            return s8 if mx is None else jnp.maximum(mx, s8)

        def pv(h, m, c, acc):
            s_r = (sa, sb)[h % 2]
            p = jnp.exp2(s_r[c * CK:(c + 1) * CK, :] - m).astype(_BF)
            o = _dot(_bf(v_s[HH * hf + h, :, c * CK:(c + 1) * CK]), p)
            return o if acc is None else acc + o

        carry = {}

        def finish_head(h, acc):
            b = 2 * DH * (h // 2)
            if h % 2 == 0:
                o = acc * (1.0 / acc[DH:DH + 1])
                o_s[b:b + 24, :] = o[0:24]
                carry["mid"] = o[24:32]
            else:
                o = acc * (1.0 / acc[0:1])
                o_s[b + 24:b + 32, :] = jnp.where(low4, carry["mid"], o[0:8])
                o_s[b + 32:b + 56, :] = o[8:32]

        def ffn_up(t):
            lo = sum(fsplit[:t])
            sl = slice(lo, lo + fsplit[t])
            n = fsplit[t]

            def wg(r0, r1):
                return _cat([w1_v[hf, r0:r1, sl], w3_v[hf, r0:r1, sl]], 1)
            z = _dot(_bf(xn_s[qb, :, 768:896]), wg(320, 448))
            ya = _dot(_bf(xn_s[qb, :, 0:384]), wg(0, 384)) + z
            yb = _dot(_bf(xn_s[qb, :, 384:768]), _cat([wg(0, 320), wg(384, 448)], 0)) + z
            for i, y in enumerate((ya, yb)):
                g = y[:, :n] * 0.5
                h_s[i * HB // 2:(i + 1) * HB // 2, sl] = _pk(g * y[:, n:] * (1.0 + jnp.tanh(g)))

        m = None
        for h in range(HH + 1):
            qm = q_head(h) if h < HH else None
            mx = acc = None
            for c in range(NC):
                for t, at in enumerate(ffn_at):
                    if at == (h, c):
                        ffn_up(t)
                if h < HH:
                    mx = qk(h, qm, c, mx)
                if h > 0:
                    acc = pv(h - 1, m, c, acc)
            if h > 0:
                finish_head(h - 1, acc)
            if h < HH:
                m = jnp.max(mx, axis=0, keepdims=True)
        for t, at in enumerate(ffn_at):
            if at is None:
                ffn_up(t)
        y = _dot(_bf(wot_s[hf]), o_s[...].astype(_BF))
        y = y + _dot_nt(w2_v[hf], _bf(h_s[...]))
        y = y + jnp.where(hf == 0, x_v[qb].astype(_F32), y_s[...])
        y_s[...] = y
        out_v[qb] = y.astype(_BF)

        @pl.when(hf == 1)
        def _():
            out_cp(qb).start()

    def body(it, c):
        half_block(it)
        return c
    lax.fori_loop(0, 2 * NQ, body, 0)
    for qb in range(NQ):
        out_cp(qb).wait()


def build(CK=128, fsplit=(256, 256, 256, 128), ffn_at=((8, 0), (8, 4), (8, 8), (8, 12)), flags=None, name="fused"):
    def fn(A_x, A_wqkv, A_wo, B_x, B_w1, B_w3, B_w2):
        del B_x
        xt = A_x.reshape(S, D).T
        any_spec = pl.BlockSpec(memory_space=pl.ANY)
        out = pl.pallas_call(
            functools.partial(_kernel, CK=CK, fsplit=fsplit, ffn_at=ffn_at),
            out_shape=jax.ShapeDtypeStruct((D, S), _BF),
            in_specs=[any_spec] * 6,
            out_specs=any_spec,
            scratch_shapes=[
                pltpu.VMEM((NQ, D, BQ), _BF),
                pltpu.VMEM((D, 3 * D), _BF),
                pltpu.VMEM((D, D), _BF),
                pltpu.VMEM((2, D, FH), _BF),
                pltpu.VMEM((2, D, FH), _BF),
                pltpu.VMEM((2, D, FH), _BF),
                pltpu.VMEM((3 * D // 2, 640), _U32),
                pltpu.VMEM((2, D // 2, 256), _U32),
                pltpu.VMEM((NQ, 448, HB), _U32),
                pltpu.VMEM((NQ, HB // 2, 896), _U32),
                pltpu.VMEM((4, S // 2, 128), _U32),
                pltpu.VMEM((2 * NQ, D // 4, BQ), _U32),
                pltpu.VMEM((H, 16, S), _U32),
                pltpu.VMEM((S, BQ), _F32),
                pltpu.VMEM((S, BQ), _F32),
                pltpu.VMEM((256, BQ), _F32),
                pltpu.VMEM((BQ // 2, FH), _U32),
                pltpu.VMEM((D, BQ), _F32),
                pltpu.VMEM((NQ, D, BQ), _BF),
                pltpu.SemaphoreType.DMA((16,)),
            ],
            compiler_params=pltpu.CompilerParams(vmem_limit_bytes=100 << 20, flags=flags),
            name=name,
        )(xt, A_wqkv, A_wo, B_w1, B_w3, B_w2.T)
        return out.T.reshape(1, S, D)
    return jax.jit(fn)


pallas_parallel_sum__softmax_full_mha__glu_gated_swiglu__prompt_kernel = build()
```

```python
import bisect
import functools
import itertools
import math

import jax
import jax.numpy as jnp
from jax import lax
import jax.experimental.pallas as pl
import jax.experimental.pallas.tpu as pltpu

_BF = jnp.bfloat16
_F32 = jnp.float32
_U32 = jnp.uint32

S, D, F, H = 2048, 448, 1792, 16
DH = D // H
BQ = 512
NQ = S // BQ
NIT = H // 2
TF = S // NIT
NU = F // 256
CK = 128
NC = S // CK
NI = 2 * NQ
EPS = 1e-5
QSCALE = 4 * DH ** -0.5 * math.log2(math.e)
SAFE = 2.0 ** 80


def _bf(x):
    return pltpu.bitcast(x, _BF)


def _u32(x):
    return pltpu.bitcast(x, _U32)


def _pk(x):
    return _u32(x.astype(_BF))


def _dot(a, b):
    return jnp.dot(a, b, preferred_element_type=_F32)


def _dot_nt(a, b):
    return lax.dot_general(a, b, (((1,), (1,)), ((), ())), preferred_element_type=_F32)


def _cat(xs, axis):
    return xs[0] if len(xs) == 1 else jnp.concatenate(xs, axis=axis)


def _tile(i, n=128):
    return slice(i * n, (i + 1) * n)


def _depth_tiles(a, b):
    zb = b[320:384].astype(_BF).astype(_F32)
    za = a[384:448].astype(_BF).astype(_F32)
    return [_cat([a[256:320], a[320:384] - zb], 0), a[0:128], a[128:256],
            b[0:128], b[128:256], _cat([b[256:320], b[384:448] - za], 0), _cat([zb, za], 0)]


def _depth_rows(w):
    return _cat([w[256:384], w[0:256], w[256:320], w[384:448], w[320:448]], 0)


def _after(never, mark, x):
    head = jnp.where(never, mark, x[0:8, 0:128])
    top = _cat([head] + ([x[0:8, 128:]] if x.shape[1] > 128 else []), 1)
    return _cat([top] + ([x[8:]] if x.shape[0] > 8 else []), 0)


def _project(wt, x, pace=_bf):
    z = _dot(_bf(wt(512, 640)), x(6, 7))
    return _cat([_dot(pace(wt(0, 384)), x(0, 3)) + z, _dot(pace(wt(128, 512)), x(3, 6)) + z], 1)


def _kernel(x_hbm, wqkv_hbm, wo_hbm, w1_hbm, w3_hbm, w2_hbm, out_hbm,
            x_v, wv_v, wqk_v, wo_v, w1_v, w3_v, w2_v,
            wt_s, wot_s, wu_s, wd_s, xt_s, xn_s, k_s, q_s, kt_s, v_s, kf_s, qf_s, qm_s, kp_s, kb_s, qb_s, p_s, pv_s, o_s, h_s,
            y_s, bad_s, kc_s, vc_s, xc_s, fc_s, m_s, out_v, sems, *, KV, loads, cap, delay, extra, lag, lead, tail, early, nfirst, lnper, wper, trips, swap, hold, nh, rot, late):
    x_cp = [pltpu.make_async_copy(x_hbm.at[:, pl.ds(c * TF, TF)], x_v.at[c], sems.at[c]) for c in range(NIT)]
    wv_cp = pltpu.make_async_copy(wqkv_hbm.at[:, pl.ds(2 * D, D)], wv_v, sems.at[8])
    wqk_cp = pltpu.make_async_copy(wqkv_hbm.at[:, pl.ds(0, 2 * D)], wqk_v, sems.at[9])
    w_cp = [pltpu.make_async_copy(src, dst, sems.at[10 + j])
            for j, (src, dst) in enumerate(((wo_hbm, wo_v), (w1_hbm, w1_v), (w3_hbm, w3_v), (w2_hbm, w2_v)))]
    out_cp = [pltpu.make_async_copy(out_v.at[c], out_hbm.at[:, pl.ds(c * TF, TF)], sems.at[14 + c]) for c in range(NIT)]

    for cp in x_cp[0:3] + [wqk_cp] + x_cp[3:] + [wv_cp] + w_cp:
        cp.start()
    for ref in (p_s, pv_s.at[0], h_s.at[0], qb_s.at[0, 0, 0], kb_s.at[0, 0], kc_s, vc_s, xc_s, fc_s, m_s.at[0], qf_s.at[0], qm_s.at[0]):
        ref[0:8, 0:128] = jnp.zeros((8, 128), ref.dtype)
    bad_s[...] = jnp.zeros(bad_s.shape, _F32)

    low4 = lax.broadcasted_iota(jnp.int32, (8, BQ), 0) < 4
    row8 = lax.broadcasted_iota(jnp.int32, (8, 128), 0)
    low = row8 < 4
    zero = jnp.zeros((8, 128), _F32)
    x_cp[0].wait()
    never0 = row8 > 8 + (_u32(x_v[0, 0:16, 0:128]) & jnp.uint32(1)).astype(jnp.int32)

    def layer_norm(blk):
        ab = []
        for t in range(2):
            x = [x_v[blk, _tile(j, 64), _tile(t)].astype(_F32) for j in range(7)]
            tot = None
            for xj in x:
                part = jnp.sum(xj.reshape(8, 8, 128), axis=0)
                tot = part if tot is None else tot + part
                yield tot
            mu = jnp.sum(tot, axis=0, keepdims=True) * (1.0 / D)
            x = [xj - mu for xj in x]
            tot = None
            for xj in x:
                part = jnp.sum((xj * xj).reshape(8, 8, 128), axis=0)
                tot = part if tot is None else tot + part
                yield tot
            rs = 0.5 * lax.rsqrt(jnp.sum(tot, axis=0, keepdims=True) * (1.0 / D) + EPS)
            ab.append(_cat([xj * rs for xj in x], 0))
        a, b = ab
        a11, a12, a21, a22 = a[0:128], a[128:256], b[0:128], b[128:256]
        sums = [a11 + a22, a21 + a22, a11 + a12, a21 - a11, a12 - a22]
        xt_s.at[blk][...] = _pk(_cat(_depth_tiles(a, b) + sums, 1))
        for j in range(8):
            yield functools.reduce(jnp.bitwise_or, [xt_s[blk, _tile(j, 8), _tile(t)] for t in range(7, 12)])

    def ffn_weights():
        for u in range(NU):
            for r in range(0, 128, 16):
                def w(k, t):
                    return _cat([w_v[k + r:k + r + 16, _tile(2 * u + t)] for w_v in (w1_v, w3_v)], 1)
                b11, b21, b12, b22 = (w(k, t).astype(_F32) for t in range(2) for k in (0, 128))
                kb = 256 if r < 64 else 320
                tiles = [b21 - b11, w(320, 0), w(0, 0), w(kb, 0), w(320, 1), b12 - b22, w(128, 1), w(256, 1),
                         b11 + b22, b21 + b22, w(256, 0), b11 + b12, w(kb, 1)]
                rows = [slice(64 * j + r // 2, 64 * j + r // 2 + 8) for j in range(13)]
                for j, t in zip(rows, tiles):
                    wu_s.at[u][j, :] = _pk(t)
                for half in range(2):
                    yield functools.reduce(jnp.bitwise_or, [wu_s[u, j, _tile(half)] for j in rows])
            for r in range(0, D // 2, 16):
                top, bot = (w2_v[k + r:k + r + 16, _tile(u, 256)].astype(_F32) for k in (0, D // 2))
                a11, a12, a21, a22 = top[:, :128], top[:, 128:], bot[:, :128], bot[:, 128:]
                rows = slice(r // 2, r // 2 + 8)
                wd_s.at[u][rows, :] = _pk(_cat([a21 + a22, a22, a21 - a11, a11 + a22, a11, a11 + a12, a12 - a22], 1))
                yield functools.reduce(jnp.bitwise_or, [wd_s[u, rows, _tile(j)] for j in (0, 2, 3, 5, 6)])

    def pacer(side, period):
        count = [0]

        def pace(x):
            parts = []
            for j in range(0, x.shape[0], 8):
                count[0] += 1
                mark = next(side, None) if count[0] // period > (count[0] - 1) // period else None
                parts.append(x[j:j + 8] if mark is None else _after(never0, _u32(mark), x[j:j + 8]))
            return _bf(_cat(parts, 0))
        return pace

    def proj(blk, i, pace):
        return _project(lambda lo, hi: wt_s[_tile(i, D // 2), lo:hi],
                        lambda lo, hi: _bf(_cat([xt_s[blk, :, _tile(j)] for j in range(lo, hi)], 0)), pace)

    def head_norms(t):
        parts = []
        for p in range(NIT):
            sq = [t[2 * DH * p + 8 * j:2 * DH * p + 8 * j + 8] for j in range(7)]
            sq = [a * a for a in sq]
            parts += [sq[0] + sq[1] + sq[2] + jnp.where(low, sq[3], 0.0),
                      sq[4] + sq[5] + sq[6] + jnp.where(low, 0.0, sq[3])]
        for step in (1, 2, 4):
            keep = (row8 & step) == 0
            parts = [jnp.where(keep, a, b) + pltpu.roll(jnp.where(keep, b, a), step, 0)
                     for a, b in zip(parts[0::2], parts[1::2])]
        return parts

    k_norm = [zero, zero]
    q_norm = []

    row2 = lax.broadcasted_iota(jnp.int32, (8, TF), 0)

    def proj_k(blk, pace):
        kt = proj(blk, 1, pace)
        for p in range(NIT):
            kp = _cat([kt[_tile(p, 2 * DH)], jnp.where((row2 == 0) | (row2 == 2), 1.0, 0.0)], 0)
            k_s[p, _tile(blk), :] = _u32(_cat([kp, jnp.zeros((64, TF), _F32)], 0).astype(_BF).T)
            if TF * blk < KV:
                kt_s.at[p][:, _tile(blk, TF)] = _pk(kp)
        for t in range(2):
            k_norm[:] = [jnp.maximum(a, b) for a, b in zip(k_norm, head_norms(kt[:, _tile(t)]))]

    def proj_v(blk, pace):
        vt = proj(blk, 2, pace)
        for p in range(NIT):
            b = 2 * DH * p
            mid = vt[b + 24:b + 32]
            v_s.at[2 * p][:, _tile(blk, TF)] = _pk(_cat([vt[b:b + 24], jnp.where(row2 < 4, mid, 1.0)], 0))
            v_s.at[2 * p + 1][:, _tile(blk, TF)] = _pk(_cat([jnp.where(row2 < 4, 1.0, mid), vt[b + 32:b + 56]], 0))

    def proj_q(blk, pace):
        qt = proj(blk, 0, pace) * QSCALE
        for p in range(NIT):
            q_s.at[p, blk // 2][:, _tile(blk % 2, TF)] = _pk(_cat([qt[_tile(p, 2 * DH)], jnp.zeros((8, TF), _F32)], 0))
        for t in range(2):
            q_norm.append(head_norms(qt[:, _tile(t)]))

    def token_tiles(blk):
        rows = [xt_s[blk, :, _tile(j)] for j in (4, 6, 1, 8, 5, 9, 0, 7, 11, 10)]
        xn_s[blk] = _u32(_bf(_cat(rows, 0)).T)

    def spread_keys(d, r0, k):
        kp_s[d, r0:r0 + 8, :] = jnp.broadcast_to(k[:, d:d + 1], (8, 128))

    list(layer_norm(0))
    x_cp[1].wait()
    list(layer_norm(1))
    x_cp[2].wait()
    list(layer_norm(2))
    first_cp = [wqk_cp]
    for cp in first_cp:
        cp.wait()
    wt_s[0:D] = _u32(_depth_rows(wqk_v[...]).T)
    proj_k(0, _bf)
    proj_k(1, _bf)
    proj_q(0, _bf)
    proj_q(1, _bf)
    second_cp = x_cp[3:] + [wv_cp]
    for cp in second_cp:
        cp.wait()
    for blk in range(2, NIT):
        side = layer_norm(blk + 1) if blk + 1 < NIT else iter(())
        pace = pacer(side, lnper)
        proj_k(blk, pace)
        proj_q(blk, pace)
        list(side)
        if blk == 2:
            for p in range(0, NIT, 4):
                kf = _cat([kt_s[p + j, :, 0:-(-KV // 128) * 128] for j in range(4)], 0).T[0:KV]
                for j in range(4):
                    kf_s[p + j] = pltpu.roll(kf, 128 - 32 * j, 1) if j else kf
            for d in range(nfirst):
                for r0 in range(0, KV, 8):
                    spread_keys(d, r0, kf_s[0, r0:r0 + 8, :])
    wt_s[D:3 * D // 2] = _u32(_depth_rows(wv_v[...]).T)
    if late:
        for cp in w_cp:
            cp.wait()
        w_cp = []
    k_max = [jnp.max(a, axis=1, keepdims=True) for a in k_norm]
    for t, norms in enumerate(q_norm):
        for j in range(2):
            shift = _u32(-jnp.sqrt(norms[j] * k_max[j])) >> 16
            for r in range(4):
                where = (4 * j + r, t // 4, slice(24, 32), _tile(t % 4))
                q_s[where] = jnp.where(low, q_s[where], shift if r == 2 else pltpu.roll(shift, (4 - 2 * r) % 8, 0))
    for cp in w_cp:
        cp.wait()
    side = ffn_weights()
    for blk in range(NIT):
        proj_v(blk, pacer(side, wper))
        token_tiles(blk)
    list(side)
    for d in range(nfirst, DH):
        for r0 in range(0, KV, 8):
            spread_keys(d, r0, kf_s[0, r0:r0 + 8, :])
    wot_s[...] = _u32(_depth_rows(wo_v[...]).T)

    def q_head(odd, w, shifted):
        none = jnp.zeros((8, BQ), _U32)
        row = lax.broadcasted_iota(jnp.int32, (8, BQ), 0)
        own = row < DH // 2 - 8
        if odd:
            last = jnp.where((row < 4) | (row == 5) if shifted else row < 4, w[24:32], none)
            return _cat([none, jnp.where(own, none, w[8:16]), w[16:24], last], 0)
        last = jnp.where(row == 4, w[24:32], none) if shifted else none
        return _cat([w[0:8], jnp.where(own, w[8:16], none), none, last], 0)

    def trip(it):
        nxt = jnp.minimum(it + 1, NIT - 1)
        never = lax.broadcasted_iota(jnp.int32, (8, 128), 0) > it + NIT

        blocks = [(r0, c0) for r0 in range(0, KV, 16) for c0 in range(2)]
        if swap:
            blocks[0:6] = sorted(blocks[0:6], key=lambda b: b[1])
        work = [(i, r0, c0, d) for i in range(NI) for r0, c0 in blocks for d in range(DH)]
        spread = [(d, r0) for d in range(DH) for r0 in range(0, KV, 8)]
        st = dict(done=0, acc=None, n=0, slot=0, qk=0, spread=0, seen=[], old=None, due=[])

        def queries(i):
            if i < NQ and i not in st["seen"]:
                st["seen"].append(i)
                w = q_s[it, i]
                qf_s[i] = _bf(w).astype(_F32)
                for odd in range(2):
                    qm_s[i + NQ * odd] = q_head(odd, w, True)

        def vpu(upto):
            while st["done"] < min(upto, len(work)):
                i, r0, c0, d = work[st["done"]]
                st["done"] += 1
                row = DH * (i // NQ) + d
                qt = 2 * (1 - d % 2)
                if r0 == 0:
                    if c0 == 0 and d == 0:
                        queries(i)
                    if d == 0 or row % 8 == 0:
                        src = [qf_s[i % NQ, _tile(row // 8, 8), _tile(2 * c0 + j)] for j in range(2)]
                        if st["old"] is not None:
                            src = [jnp.where(never, st["old"], x) for x in src]
                        st["src"] = _cat(src, 1)
                    qb_s[i % 2, d // 2, c0, :, 128 * qt:128 * qt + 256] = jnp.broadcast_to(
                        st["src"][row % 8:row % 8 + 1], (8, 256))
                    if c0 == 0 and d == 0:
                        qb_s[i % 2, DH // 2, 0] = jnp.broadcast_to(qf_s[i % NQ, _tile(2 * DH + 2 * (i // NQ), 1)], (8, BQ))
                ks = []
                for r in range(2):
                    if i % NQ == 0 and c0 == 0:
                        kp = kp_s[row // 2, r0 + 8 * r:r0 + 8 * r + 8, :]
                        ks.append(pltpu.bitcast(kp & jnp.uint32(0xFFFF0000) if row % 2 else kp << 16, _F32))
                        kb_s[row // 2, r0 // 16, :, _tile(2 - qt + r)] = ks[-1]
                    else:
                        ks.append(kb_s[row // 2, r0 // 16, :, _tile(2 - qt + r)])
                qs = [qb_s[i % 2, d // 2, c0, :, _tile(qt + j)] for j in range(2)]
                if d == 0:
                    st["acc"] = [qb_s[i % 2, DH // 2, 0, :, _tile(2 * c0 + j)] for j in range(2)] * 2
                acc = st["acc"] = [a + t for a, t in zip(st["acc"], [k * q for k in ks for q in qs])]
                if d % 7 == 3:
                    st["old"] = acc[0]
                if d == DH - 1:
                    s = _cat([_cat(acc[0:2], 1), _cat(acc[2:4], 1)], 0)
                    p = jnp.exp2(s)
                    pv_s.at[i][r0 // 2:r0 // 2 + 8, _tile(c0, 256)] = _pk(p)
                    if hold >= 0:
                        st["due"] += [None] * hold + [_u32(p[8:16, 128:256])]

        def paced(x):
            parts = []
            for j in range(0, x.shape[0], 8):
                xj = x[j:j + 8]
                slot = st["slot"]
                st["slot"] += 1
                if target[slot] > 0 and st["done"] < len(work):
                    vpu(target[slot])
                    mark = st["due"].pop(0) if st["due"] else None
                    for _ in range(nh):
                        a = _u32(st["acc"][rot[st["n"] % len(rot)]])
                        mark = a if mark is None else mark | a
                        st["n"] += 1
                    head = jnp.where(never, mark, xj[:, 0:128])
                    xj = head if x.shape[1] == 128 else _cat([head, xj[:, 128:]], 1)
                parts.append(xj)
            return _bf(_cat(parts, 0))

        def cached(first, copy, src, idx, *sl):
            if first:
                x = src[(idx,) + sl]
                copy[sl] = x
                return x
            return copy[sl]

        def qk(i, lo, hi):
            queries(i)
            k = paced(cached(i == 0, kc_s, k_s, it, slice(lo // 2, hi // 2), slice(None)))
            s = _dot(k, _bf(_cat([qm_s[i], jnp.zeros((32, BQ), _U32)], 0)))
            p_s[lo // 2:hi // 2, :] = _pk(jnp.exp2(s))
            for j in range(0, hi - lo, 8):
                st["qk"] += 8
                pos = st["qk"] / (S - KV)
                goal = len(spread) / 2 * ((pos - 1.1) / 4 if pos < 5.1 else 1 + (pos - 5.1) / 2.9)
                while st["spread"] < min(goal, len(spread)):
                    d, r0 = spread[st["spread"]]
                    vpu((1 + NQ * (d >= DH // 2)) * len(work) // NI)
                    k = cached(d == 0, fc_s, kf_s, nxt, slice(r0, r0 + 8), slice(None))
                    spread_keys(d, r0, jnp.where(never, _u32(s[j:j + 8, 0:128]), k))
                    st["spread"] += 1

        def pv(i, lo, hi, last):
            parts = []
            if lo < KV:
                vpu((i * KV + min(hi, KV)) * len(work) // (NI * KV))
                parts.append(pv_s[i, lo // 2:min(hi, KV) // 2, :])
            if hi > KV:
                parts.append(p_s[max(lo, KV) // 2:hi // 2, :])
            v = cached(i % NQ == 0, vc_s, v_s, 2 * it + i // NQ, slice(None), slice(lo, hi))
            o = _dot(paced(v), _bf(_cat(parts, 0)))
            st["o"] = o if hi == S else st["o"] + o
            if last:
                o_s[it, _tile(i // NQ, 32), _tile(i % NQ, BQ)] = st["o"]
                den = st["o"][0:8] if i >= NQ else st["o"][24:32]
                bad_s[i // NQ] = jnp.where((den >= 1.0 / SAFE) & (den <= SAFE), bad_s[i // NQ], 1.0)

        def ffn_up(u, part):
            def x(j, first=True):
                return cached(u == 0 and first, xc_s, xn_s, it, slice(None), _tile(j))

            def w(j, n=1):
                return _bf(wu_s[u, 64 * j:64 * (j + n)])

            def act(y):
                g = y[:, 0:128]
                return g * y[:, 128:256] * (1.0 + jnp.tanh(g))
            if part == 0:
                st["m4"] = _dot(paced(_cat([x(0), x(1)], 1)), w(0, 2))
            elif part == 1:
                st["m2"] = _dot(paced(x(3)), w(2))
                st["h12"] = act(st["m4"] + st["m2"] + _dot(_bf(x(4)), w(3)))
            elif part == 2:
                st["m3"] = _dot(paced(_cat([x(1, False), x(2)], 1)), w(4, 2))
            elif part == 3:
                m5 = _dot(paced(x(5)), w(6))
                st["h21"] = act(st["m3"] + m5 + _dot(_bf(x(6)), w(7)))
                st["m4"] = st["m4"] - m5
                st["m3"] = st["m3"] - st["m2"]
            elif part == 4:
                a = x(7)
                st["m1"] = _cat([_dot(paced(a[0:32]), w(8)), _dot(_bf(a[32:64]), w(8))], 0)
            elif part == 5:
                h11 = st["h11"] = act(st["m1"] + st["m4"] + _dot(paced(_cat([x(8), x(6, False)], 1)), w(9, 2)))
                h_s.at[u][:, 0:384] = _pk(_cat([h11, st["h21"] - h11, h11 + st["h12"]], 1))
            else:
                h22 = act(st["m1"] + st["m3"] + _dot(paced(_cat([x(9), x(4, False)], 1)), w(11, 2)))
                h_s.at[u][:, 384:896] = _pk(_cat([st["h11"] + h22, st["h12"] - h22, h22, st["h21"] + h22], 1))

        def ffn_down(lo, hi):
            def put(r, t, y):
                y_s[it, _tile(r, D // 2), _tile(t)] = y
            first = True
            mark = _u32(st["acc"][0])
            while lo < hi:
                n, k0 = divmod(lo, NU)
                i = (1, 3, 2, 4, 0, 6, 5)[n]
                k1 = min(NU, k0 + hi - lo)
                col = _tile((3, 0, 4, 1, 5, 2, 6)[i])
                a = _cat([wd_s[k, :, col] for k in range(k0, k1)], 1)
                b = _bf(_cat([h_s[k, :, col] for k in range(k0, k1)], 1))
                if hi == 1:
                    y = _cat([_dot_nt(paced(a[0:32]), b), _dot_nt(_bf(a[32:64]), b),
                              _dot_nt(_bf(a[64:96]), b), _dot_nt(_bf(a[80:112]), b)[32:64]], 0)
                elif first:
                    y = _dot_nt(paced(a), b)
                else:
                    head = [jnp.where(never, mark, a[0:8, _tile(j)]) for j in range(k1 - k0)]
                    y = _dot_nt(_bf(_cat([_cat(head, 1), a[8:]], 0)), b)
                y = y if k0 == 0 else m_s[i] + y
                lo += k1 - k0
                first = False
                if k1 < NU or i < 5:
                    m_s[i] = y
                if k1 == NU:
                    if i == 3:
                        put(1, 0, m_s[1] + y)
                    elif i == 4:
                        put(0, 1, m_s[2] + y)
                    elif i == 6:
                        put(0, 0, m_s[0] + m_s[3] - m_s[4] + y)
                    elif i == 5:
                        put(1, 1, m_s[0] - m_s[1] + m_s[2] + y)

        nv = -(-KV // CK)
        order = list(range(NC - 1, nv - 1, -1)) + list(range(nv))
        seq = [(i, c) for i in range(NI) for c in order]
        ffn = []
        for u in range(NU):
            ups = [(functools.partial(ffn_up, u, part), 4 if part == 4 else 8, ld + loads[2])
                   for part, ld in enumerate((4, 16, 4, 24, 0, 27, 30))]
            ffn += [ups[0:2], ups[2:5], ups[5:7]]
        ffn += [[(functools.partial(ffn_down, 0, 1), 4, loads[3]), (functools.partial(ffn_down, 1, 5), 14, loads[3])]]
        ffn += [[(functools.partial(ffn_down, lo, lo + 4), 14, loads[3])] for lo in range(5, 49, 4)]
        tape = []
        nf = 0
        for t in range(len(seq) + lag):
            if t < len(seq):
                i, c = seq[t]
                lo, hi = max(c * CK, KV), (c + 1) * CK
                if hi > lo:
                    tape.append((functools.partial(qk, i, lo, hi), (hi - lo) // 16, loads[0]))
            while nf < len(ffn) and ((nf + 1 - early) * len(seq) <= (t + 1) * len(ffn) if nf + 1 < len(ffn)
                                     else t + 1 >= len(seq)):
                tape += ffn[nf]
                nf += 1
            if t >= lag:
                i, c = seq[t - lag]
                last = c == order[-1]
                tape.append((functools.partial(pv, i, c * CK, (c + 1) * CK, last), 2, loads[4] if last else loads[1]))
        load = [0] * delay + [ld for _, n, ld in tape for _ in range(n)]
        nslot = len(load) - delay
        share = [0 if t < lead or t >= nslot - tail else cap - load[t] for t in range(nslot)]
        cost = [0]
        for i, r0, c0, d in work:
            cost.append(cost[-1] + 8 + extra[0] * (i % NQ == 0 and c0 == 0) + extra[2] * (i == 0 and r0 < 48) + extra[1] * (r0 == 0) + 6 * (d == DH - 1))
        target, run = [], 0
        for w in share:
            run += w
            target.append(min(len(work), bisect.bisect_left(cost, cost[-1] * run / sum(share))))
        for step, _, _ in tape:
            step()
        assert st["slot"] == nslot and st["spread"] == len(spread) and st["done"] == len(work)

    def body(it, c):
        if trips:
            trip(it)
        else:
            o_s[it, 0:8, 0:128] = sum(pltpu.bitcast(r[(it,) + (0,) * (len(r.shape) - 3) + (slice(0, 8), slice(0, 128))], _F32) for r in (wu_s, wd_s, xn_s, k_s, q_s, v_s, kf_s, kp_s))
        return c
    lax.fori_loop(0, NIT, body, 0)

    @pl.when(jnp.max(jnp.where(low4, bad_s[1], bad_s[0])) > 0.0)
    def _():
        def exact(n, carry):
            pair, c = n // NQ, n % NQ
            cols = pl.ds(pl.multiple_of(c * BQ, BQ), BQ)
            for odd in range(2):
                h = 2 * pair + odd
                qm = _bf(_cat([q_head(odd, q_s[pair, c], False), jnp.zeros((32, BQ), _U32)], 0))

                def scores(j):
                    k = _bf(k_s[pair, pl.ds(pl.multiple_of(j * (CK // 2), CK // 2), CK // 2), :])
                    return _dot(k, qm)
                mx = lax.fori_loop(0, NC, lambda j, a: jnp.maximum(a, jnp.max(scores(j), axis=0, keepdims=True)),
                                   jnp.full((1, BQ), -jnp.inf, _F32))

                def add(j, acc):
                    p = jnp.exp2(scores(j) - mx).astype(_BF)
                    return acc + _dot(_bf(v_s[h, :, pl.ds(pl.multiple_of(j * CK, CK), CK)]), p)
                o_s[pair, _tile(odd, 32), cols] = lax.fori_loop(0, NC, add, jnp.zeros((32, BQ), _F32))
            return carry
        lax.fori_loop(0, NIT * NQ, exact, 0)

    def attended(t):
        rows = []
        for p in range(NIT):
            o = o_s[p, :, _tile(t)]
            inv = 1.0 / jnp.where(low, o[32:40], o[24:32])
            even, odd = inv[4:5], inv[0:1]
            rows += [o[0:24] * even, jnp.where(low, o[24:32] * even, o[32:40] * odd), o[40:64] * odd]
        return _cat(rows, 0)

    for blk in range(NIT):
        ot = _depth_tiles(attended(2 * blk), attended(2 * blk + 1))
        y = _project(lambda lo, hi: wot_s[:, lo:hi], lambda lo, hi: _cat(ot[lo:hi], 0).astype(_BF))
        out_v[blk] = (2.0 * (y + y_s[blk]) + x_v[blk].astype(_F32)).astype(_BF)
        out_cp[blk].start()
    for cp in out_cp:
        cp.wait()


def build(KV=304, loads=(12, 9, 5, 9, 16), cap=59, delay=10, extra=(2.4, 4, 3), lag=3, lead=1, tail=4, early=2.0, nfirst=7, lnper=3, wper=2.1, trips=True, swap=1, hold=-1, nh=1, late=0, rot=(2, 3),
          flags=None, name="fused"):
    def fn(A_x, A_wqkv, A_wo, B_x, B_w1, B_w3, B_w2):
        del B_x
        xt = A_x.reshape(S, D).T
        any_spec = pl.BlockSpec(memory_space=pl.ANY)
        out = pl.pallas_call(
            functools.partial(_kernel, KV=KV, loads=loads, cap=cap, delay=delay, extra=extra, lag=lag, lead=lead,
                              tail=tail, early=early, nfirst=nfirst, lnper=lnper, wper=wper, trips=trips, swap=swap, hold=hold, nh=nh, rot=rot, late=late),
            out_shape=jax.ShapeDtypeStruct((D, S), _BF),
            in_specs=[any_spec] * 6,
            out_specs=any_spec,
            scratch_shapes=[
                pltpu.VMEM((NIT, D, TF), _BF),
                pltpu.VMEM((D, D), _BF),
                pltpu.VMEM((D, 2 * D), _BF),
                pltpu.VMEM((D, D), _BF),
                pltpu.VMEM((D, F), _BF),
                pltpu.VMEM((D, F), _BF),
                pltpu.VMEM((D, F), _BF),
                pltpu.VMEM((3 * D // 2, 640), _U32),
                pltpu.VMEM((D // 2, 640), _U32),
                pltpu.VMEM((NU, 13 * 64, 256), _U32),
                pltpu.VMEM((7, D // 4, F // 2), _U32),
                pltpu.VMEM((NIT, 64, 12 * 128), _U32),
                pltpu.VMEM((NIT, 64, 1280), _U32),
                pltpu.VMEM((NIT, S // 2, 128), _U32),
                pltpu.VMEM((NIT, NQ, 32, BQ), _U32),
                pltpu.VMEM((NIT, 32, -(-KV // TF) * TF), _U32),
                pltpu.VMEM((H, 16, S), _U32),
                pltpu.VMEM((NIT, KV, 128), _U32),
                pltpu.VMEM((NQ, 64, BQ), _F32),
                pltpu.VMEM((NI, 32, BQ), _U32),
                pltpu.VMEM((DH, KV, 128), _U32),
                pltpu.VMEM((DH, KV // 16, 8, 512), _F32),
                pltpu.VMEM((2, DH // 2 + 1, 2, 8, 512), _F32),
                pltpu.VMEM((S // 2, BQ), _U32),
                pltpu.VMEM((NI, KV // 2, BQ), _U32),
                pltpu.VMEM((NIT, 64, S), _F32),
                pltpu.VMEM((7, 64, F // 2), _U32),
                pltpu.VMEM((NIT, D, TF), _F32),
                pltpu.VMEM((2, 8, BQ), _F32),
                pltpu.VMEM((S // 2, 128), _U32),
                pltpu.VMEM((16, S), _U32),
                pltpu.VMEM((64, 1280), _U32),
                pltpu.VMEM((KV, 128), _U32),
                pltpu.VMEM((7, D // 2, 128), _F32),
                pltpu.VMEM((NIT, D, TF), _BF),
                pltpu.SemaphoreType.DMA((22,)),
            ],
            compiler_params=pltpu.CompilerParams(vmem_limit_bytes=100 << 20, flags=flags),
            name=name,
        )(xt, A_wqkv, A_wo, B_w1, B_w3, B_w2.T)
        return out.T.reshape(1, S, D)
    return jax.jit(fn)


pallas_parallel_sum__softmax_full_mha__glu_gated_swiglu__prompt_kernel = build()
```

```python
import bisect
import functools
import math

import jax
import jax.numpy as jnp
from jax import lax
import jax.experimental.pallas as pl
import jax.experimental.pallas.tpu as pltpu

_BF = jnp.bfloat16
_F32 = jnp.float32
_U32 = jnp.uint32

S, D, F, H = 2048, 448, 1792, 16
DH = D // H
BQ = 512
NQ = S // BQ
NIT = H // 2
NI = 2 * NQ
NU = F // 256
CK = 128
NC = S // CK
KV = 304
NX = 25
LAG = 3
EPS = 1e-5
QSCALE = 4 * DH ** -0.5 * math.log2(math.e)
HUGE, TINY = 2.0 ** 120, 2.0 ** -8


def _bf(x):
    return pltpu.bitcast(x, _BF)


def _u32(x):
    return pltpu.bitcast(x, _U32)


def _pk(x):
    return _u32(x.astype(_BF))


def _dot(a, b):
    return jnp.dot(a, b, preferred_element_type=_F32)


def _dot_nt(a, b):
    return lax.dot_general(a, b, (((1,), (1,)), ((), ())), preferred_element_type=_F32)


def _cat(xs, axis):
    return xs[0] if len(xs) == 1 else jnp.concatenate(xs, axis=axis)


def _tile(i, n=128):
    return slice(i * n, (i + 1) * n)


def _merge(marks):
    return functools.reduce(jnp.bitwise_or, marks)


def _after(never, mark, x):
    head = lax.select(never, mark, x[:, 0:128])
    return head if x.shape[1] == 128 else _cat([head, x[:, 128:]], 1)


def _token_operands(x):
    short, long = [], []
    for t in (0, 2):
        a, b = ([x(t + i, j) for j in range(7)] for i in range(2))
        short.append([b[3:6], a[0:3], [a[j] + b[3 + j] for j in range(3)]])
        long.append([[b[j] + b[3 + j] for j in range(3)] + [b[6]], [a[j] + a[3 + j] for j in range(3)] + [a[6]],
                     [a[3 + j] - b[3 + j] for j in range(3)] + [a[6]], [b[j] - a[j] for j in range(3)] + [b[6]]])
    ops = []
    for p, q in zip(*short):
        zq = q[1].astype(_BF).astype(_F32)
        zp = p[2].astype(_BF).astype(_F32)
        ops += [(p[0], p[1] - zq), (q[0], q[2] - zp), (zq, zp)]
    for p, q in zip(*long):
        ops += [p[0:2], p[2:4], q[0:2], q[2:4]]
    return ops


def _project(w_ref, x, cuts, pace=_bf):
    c11, c12, c21, c22 = [], [], [], []
    for lo, hi in zip(cuts, cuts[1:]):
        def w(j, n):
            return w_ref[lo // 2:hi // 2, 128 * j:128 * (j + n)]

        def short(n):
            z = _dot(_bf(w(3 * n + 2, 1)), x(3 * n + 2))
            return _cat([_dot(_bf(w(3 * n + j, 1)), x(3 * n + j)) + z for j in range(2)], 1)

        def long(n, j):
            t = [x(9 + 4 * n + i) for i in range(4)]
            return _dot(pace(w(j, 2)), _cat([_cat(t[0:2], 0), _cat(t[2:4], 0)], 1))
        m4 = short(0)
        m2 = long(0, 13)
        m3 = short(1)
        m5 = long(1, 15)
        m1 = short(2)
        c21.append(m4 + m2)
        c12.append(m3 + m5)
        c11.append(m1 + (m4 - m5) + long(2, 9))
        c22.append(m1 + (m3 - m2) + long(3, 11))
    a, b = _cat(c11 + c12, 0), _cat(c21 + c22, 0)
    return _cat([a[:, :128], b[:, :128], a[:, 128:], b[:, 128:]], 1)


def _kernel(x_hbm, wqkv_hbm, wo_hbm, w1_hbm, w3_hbm, w2_hbm, out_hbm,
            x_v, wv_v, wqk_v, wo_v, w1_v, w3_v, w2_v, out_v, last_v,
            wt_s, wu_s, wd_s, xt_s, xn_s, k_s, q_s, v_s, kt_s, kf_s, o_s, y_s, bad_s,
            kc_s, vc_s, xc_s, fc_s, qf_s, qm_s, kp_s, kb_s, qb_s, p_s, pv_s, h_s, m_s, sems):
    x_cp = [pltpu.make_async_copy(x_hbm.at[:, pl.ds(c * BQ, BQ)], x_v.at[c], sems.at[min(c, 2)]) for c in range(NQ)]
    wv_cp = pltpu.make_async_copy(wqkv_hbm.at[:, pl.ds(2 * D, D)], wv_v, sems.at[2])
    wqk_cp = pltpu.make_async_copy(wqkv_hbm.at[:, pl.ds(0, 2 * D)], wqk_v, sems.at[3])
    w_cp = [pltpu.make_async_copy(src, dst, sems.at[4])
            for src, dst in ((wo_hbm, wo_v), (w1_hbm, w1_v), (w3_hbm, w3_v), (w2_hbm, w2_v))]
    for cp in x_cp[0:2] + [wqk_cp] + x_cp[2:] + [wv_cp] + w_cp:
        cp.start()
    for ref in (p_s, pv_s.at[0], h_s.at[0], qb_s.at[0, 0, 0, 0, 0], kb_s.at[0, 0, 0, 0, 0], vc_s, xc_s, fc_s,
                m_s.at[0], qf_s.at[0], qm_s.at[0]):
        ref[0:8, 0:128] = jnp.zeros((8, 128), ref.dtype)
    bad_s[...] = jnp.zeros(bad_s.shape, _F32)
    row = lax.broadcasted_iota(jnp.int32, (8, BQ), 0)
    row8 = lax.broadcasted_iota(jnp.int32, (8, 128), 0)
    x_cp[0].wait()
    never0 = row8 > 8 + (_u32(x_v[0, 0:16, 0:128]) & jnp.uint32(1)).astype(jnp.int32)

    def layer_norm(c):
        def load(r, mark=None):
            x = x_v[c, r:r + 16]
            if mark is not None:
                x = _bf(lax.select(_cat([never0] * 4, 1), _u32(mark), _u32(x)))
            return x.astype(_F32)

        def mean(term):
            tot = None
            for r in range(0, D, 16):
                t = term(r)
                tot = t[0:8] + t[8:16] if tot is None else tot + t[0:8] + t[8:16]
                yield _u32(tot[:, _tile(r // 16 % 4)])
            return jnp.broadcast_to(jnp.sum(tot, axis=0, keepdims=True) * (1.0 / D), (8, BQ))
        mu = yield from mean(load)
        mu2 = _cat([mu, mu], 0)
        var = yield from mean(lambda r: jnp.square(load(r, mu) - mu2))
        scale = 0.5 * lax.rsqrt(var + EPS)
        for r in range(0, 64, 16):
            xn = [(load(64 * j + r, scale) - mu2) * _cat([scale, scale], 0) for j in range(7)]
            ops = _token_operands(lambda t, j: xn[j][:, _tile(t)])
            for half in range(2):
                rows = slice(32 * half + r // 2, 32 * half + r // 2 + 8)
                xt_s.at[c][rows, :] = _pk(_cat([op[half] for op in ops], 1))
                for j in range(0, NX, 5):
                    yield _merge([xt_s[c, rows, _tile(t)] for t in range(j, j + 5)])

    def transposed_weights(w, first):
        blocks = ((0, 1), (0, 2), (1, 2), (2, 6), (3, 4), (3, 5), (4, 5), (5, 6))
        wt = _cat([w[_tile(j, 64)] for pair in blocks for j in pair], 0).T
        for i in range(w.shape[1] // D):
            one, two = wt[_tile(2 * i, D // 2)], wt[_tile(2 * i + 1, D // 2)]
            b11, b21, b12, b22 = (b.astype(_F32) for b in (one[:, :512], one[:, 512:], two[:, :512], two[:, 512:]))

            def ends(b):
                return _cat([b[:, :128], b[:, 384:]], 1)
            wt_s.at[first + i][:, 0:13 * 128] = _pk(_cat([
                b21[:, :384] - b11[:, :384], b12[:, :384] - b22[:, :384], b11[:, :384] + b22[:, :384],
                ends(b21) + ends(b22), ends(b11) + ends(b12)], 1))
            wt_s[first + i, :, 13 * 128:] = _u32(_cat([ends(one[:, :512]), ends(two[:, 512:])], 1))

    def ffn_weights():
        for u in range(NU):
            def w(r, t):
                return _cat([w_v[r:r + 16, _tile(2 * u + t)] for w_v in (w1_v, w3_v)], 1)
            for r in range(0, 256, 16):
                if r < 192:
                    b11, b21, b12, b22 = (w(k + r, t).astype(_F32) for t in range(2) for k in (0, 192))
                    ops = ((0, b21 - b11), (192, b12 - b22), (384, b11 + b22), (576, b21 + b22), (832, b11 + b12),
                           (1024, w(r, 0)), (1280, w(192 + r, 1)))
                else:
                    ops = ((576, w(192 + r, 0).astype(_F32) + w(192 + r, 1).astype(_F32)),
                           (1024, w(192 + r, 0)), (1280, w(192 + r, 1)))
                rows = [slice((j + r) // 2, (j + r) // 2 + 8) for j, _ in ops]
                for j, (_, t) in zip(rows, ops):
                    wu_s.at[u][j, :] = _pk(t)
                mark = _merge([wu_s[u, j, :] for j in rows])
                if r < 192:
                    yield mark[:, :128]
                    yield mark[:, 128:]
                else:
                    yield mark[:, :128] | mark[:, 128:]
            for r in range(0, D // 2, 16):
                top, bot = (w2_v[k + r:k + r + 16, _tile(u, 256)].astype(_F32) for k in (0, D // 2))
                a11, a12, a21, a22 = top[:, :128], top[:, 128:], bot[:, :128], bot[:, 128:]
                rows = slice(r // 2, r // 2 + 8)
                wd_s.at[u][rows, :] = _pk(_cat([a21 + a22, a22, a21 - a11, a11 + a22, a11, a11 + a12, a12 - a22], 1))
                yield _merge([wd_s[u, rows, _tile(j)] for j in (0, 2, 3, 5, 6)])

    def pacer(side, period):
        count = [0]

        def pace(x):
            parts = []
            for j in range(0, x.shape[0], 8):
                count[0] += 1
                marks = [next(side, None) for _ in range(int(count[0] / period) - int((count[0] - 1) / period))]
                marks = [m for m in marks if m is not None]
                parts.append(_after(never0, _merge(marks), x[j:j + 8]) if marks else x[j:j + 8])
            return _bf(_cat(parts, 0))
        return pace

    def proj(c, i, pace):
        return _project(wt_s.at[i], lambda j: _bf(xt_s[c, :, _tile(j)]), (0, 64, 112, 176, 224), pace)

    def proj_q(c, pace):
        qt = proj(c, 0, pace) * QSCALE
        for p in range(NIT):
            q_s.at[p, c][...] = _pk(_cat([qt[_tile(p, 2 * DH)], jnp.zeros((8, BQ), _F32)], 0))

    centre = []

    def proj_k(c, pace):
        kt = proj(c, 1, pace)
        if c == 0:
            centre.append(jnp.broadcast_to(jnp.sum(kt[:, _tile(1)], axis=1, keepdims=True) * (1.0 / 128), (D, 128)))
        kt = kt - _cat(centre * 4, 1)
        for p in range(NIT):
            kp = _cat([kt[_tile(p, 2 * DH)], jnp.zeros((8, BQ), _F32)], 0)
            keys = _u32(_cat([kp, jnp.zeros((64, BQ), _F32)], 0).astype(_BF).T)
            k_s[p, _tile(c, BQ // 2), :] = keys
            if p == 0:
                kc_s[_tile(c, BQ // 2), :] = keys
            if c == 0:
                kt_s.at[p][...] = _pk(kp)

    def proj_v(c, pace):
        vt = proj(c, 2, pace)
        for p in range(NIT):
            b = 2 * DH * p
            mid = vt[b + 24:b + 32]
            v_s.at[2 * p][:, _tile(c, BQ)] = _pk(_cat([vt[b:b + 24], jnp.where(row < 4, mid, 1.0)], 0))
            v_s.at[2 * p + 1][:, _tile(c, BQ)] = _pk(_cat([jnp.where(row < 4, 1.0, mid), vt[b + 32:b + 56]], 0))

    def token_rows(c):
        xn = _u32(_bf(_cat([xt_s[c, :, _tile(j)] for j in range(NX)], 0)).T)
        xn_s[2 * c] = xn[0:32]
        xn_s[2 * c + 1] = xn[32:64]

    def spread_keys(d, r0, k):
        kp_s[d // (DH // 2), r0 // 16, d % (DH // 2), r0 // 8 % 2, 0] = jnp.broadcast_to(k[:, d:d + 1], (8, 128))

    list(layer_norm(0))
    x_cp[1].wait()
    list(layer_norm(1))
    wqk_cp.wait()
    transposed_weights(wqk_v[...], 0)
    proj_q(0, _bf)
    proj_q(1, _bf)
    for cp in x_cp[2:] + [wv_cp]:
        cp.wait()
    for c in range(1, NQ):
        side = layer_norm(c + 1) if c + 1 < NQ else iter(())
        pace = pacer(side, 1.1)
        if c == 1:
            proj_k(0, pace)
        proj_k(c, pace)
        if c > 1:
            proj_q(c, pace)
        list(side)
        if c == 1:
            token_rows(0)
            for p in range(0, NIT, 4):
                kf = _cat([kt_s[p + j, :, 0:-(-KV // 128) * 128] for j in range(4)], 0).T[0:KV]
                for j in range(4):
                    kf_s[p + j] = pltpu.roll(kf, 128 - 32 * j, 1) if j else kf
            for d in range(DH // 2):
                for r0 in range(0, KV, 8):
                    spread_keys(d, r0, kf_s[0, r0:r0 + 8, :])
    transposed_weights(wv_v[...], 2)
    for cp in w_cp:
        cp.wait()
    side = ffn_weights()
    pace = pacer(side, 0.75)
    for c in range(NQ):
        proj_v(c, pace)
        if c > 0:
            token_rows(c)
    list(side)
    for d in range(DH // 2, DH):
        for r0 in range(0, KV, 8):
            spread_keys(d, r0, kf_s[0, r0:r0 + 8, :])
    transposed_weights(wo_v[...], 3)

    def trip(it, carry):
        nxt = jnp.minimum(it + 1, NIT - 1)
        never = row8 > it + NIT
        work = [(i, r, c0, d) for i in range(NI) for r in range(KV // 16) for c0 in range(2) for d in range(DH)]
        spread = [(d, r0) for d in range(0, DH, 2) for r0 in range(0, KV, 8)]
        st = dict(done=0, slot=0, qk=0, spread=0, seen=0, old=None, src=(None, None))

        def queries(i):
            if i == st["seen"] < NQ:
                st["seen"] += 1
                w = q_s[it, i]
                qf_s[i] = _bf(w).astype(_F32)[0:2 * DH]
                even_rows = row < DH // 2 - 8
                qm_s[i, 0:16] = _cat([w[0:8], jnp.where(even_rows, w[8:16], jnp.uint32(0))], 0)
                qm_s[i + NQ] = _cat([jnp.where(even_rows, jnp.uint32(0), w[8:16]), w[16:32]], 0)

        def vpu(upto):
            while st["done"] < min(upto, len(work)):
                i, r, c0, d = work[st["done"]]
                st["done"] += 1
                odd = i // NQ
                if r == 0:
                    queries(i)
                    j = DH * odd + 2 * (d % (DH // 2)) + d // (DH // 2)
                    if st["src"][0] != (i, c0, j // 8):
                        src = qf_s[i % NQ, _tile(j // 8, 8), _tile(c0, 256)]
                        if st["old"] is not None:
                            src = lax.select(_cat([never] * 2, 1), _cat([st["old"][0, 0]] * 2, 1), src)
                        st["src"] = (i, c0, j // 8), src
                    q = jnp.broadcast_to(st["src"][1][j % 8:j % 8 + 1], (8, 256))
                    qb_s[i % 2, c0, d + 1, 0, 0] = q[:, :128]
                    qb_s[i % 2, c0, d + 1, 0, 1] = q[:, 128:]
                if i % NQ == 0 and c0 == 0:
                    kp = kp_s[odd, r, d % (DH // 2)]
                    k = lax.bitcast_convert_type(kp << 16 if d < DH // 2 else kp & jnp.uint32(0xFFFF0000), _F32)
                    kb_s[odd, r, d] = k
                else:
                    k = kb_s[odd, r, d]
                t = k * qb_s[i % 2, c0, d + 1]
                if d:
                    st["old"] = st["acc"]
                acc = st["acc"] = st["acc"] + t if d else t
                if d == DH - 1:
                    s = _cat([_cat([acc[j, 0], acc[j, 1]], 1) for j in range(2)], 0)
                    pv_s.at[i][_tile(r, 8), _tile(c0, 256)] = _pk(jnp.exp2(s))

        def paced(x):
            parts = []
            for j in range(0, x.shape[0], 8):
                upto = target[st["slot"]]
                st["slot"] += 1
                if upto > 0 and st["done"] < len(work):
                    vpu(upto)
                    parts.append(_after(never, _u32(st["acc"][1, 1]), x[j:j + 8]))
                else:
                    parts.append(x[j:j + 8])
            return _bf(_cat(parts, 0))

        def cached(first, copy, src, idx, *sl):
            if first:
                x = src[(idx,) + sl]
                copy[sl] = x
                return x
            return copy[sl]

        def qk(i, lo, hi):
            queries(i)
            odd = i // NQ
            none = [jnp.zeros((8, BQ), _U32)]
            qm = _cat(none * odd + [qm_s[i, 0:16 + 8 * odd]] + none * (6 - 2 * odd), 0)
            s = _dot(paced(kc_s[lo // 2:hi // 2]), _bf(qm))
            p_s[lo // 2:hi // 2, :] = _pk(jnp.exp2(s))
            for j in range(0, hi - lo, 8):
                st["qk"] += 8
                pos = st["qk"] / (S - KV)
                goal = len(spread) / 2 * ((pos - 1.1) / 4 if pos < 5.1 else 1 + (pos - 5.1) / 2.9)
                while st["spread"] < min(goal, len(spread)):
                    d, r0 = spread[st["spread"]]
                    st["spread"] += 1
                    vpu((1 + NQ * (d >= DH // 2)) * len(work) // NI)
                    k = cached(d == 0, fc_s, kf_s, nxt, slice(r0, r0 + 8), slice(None))
                    k = _after(never, _u32(s[j:j + 8, 0:128]), k)
                    spread_keys(d, r0, k)
                    spread_keys(d + 1, r0, k)

        def pv(i, lo, hi, last):
            parts = []
            if lo < KV:
                vpu((i * KV + min(hi, KV)) * len(work) // (NI * KV))
                parts.append(pv_s[i, lo // 2:min(hi, KV) // 2, :])
            if hi > KV:
                parts.append(p_s[max(lo, KV) // 2:hi // 2, :])
            v = cached(i % NQ == 0, vc_s, v_s, 2 * it + i // NQ, slice(None), slice(lo, hi))
            o = _dot(paced(v), _bf(_cat(parts, 0)))
            o = st["o"] = o if hi == S else st["o"] + o
            if last:
                o_s[2 * it + i // NQ, i % NQ] = o
                den, value_rows = (o[0:8], row >= 4) if i >= NQ else (o[24:32], row < 4)
                rest = o[8:16] + o[16:24] + (o[24:32] if i >= NQ else o[0:8])
                safe = (jnp.abs(rest) + jnp.abs(den) <= HUGE) & ((den >= TINY) | value_rows)
                bad_s[...] = jnp.where(safe, bad_s[...], 1.0)

        def ffn_up(u, part):
            def x(j, n=1):
                return cached(u == 0, xc_s, xn_s, it, slice(None), slice(128 * j, 128 * (j + n)))

            def w(*blocks):
                return _bf(_cat([wu_s[u, _tile(j, 32)] for j in blocks], 0))

            def short(n, z):
                return _cat([_dot(paced(x(3 * n)), w(3 * n, 3 * n + 1)) + z,
                             _dot(_bf(x(3 * n + 1)), w(3 * n, 3 * n + 2)) + z], 0)

            def long(n, *blocks):
                return _dot(paced(_cat([x(9 + 4 * n, 2), x(11 + 4 * n, 2)], 0)), w(*blocks))

            def act(y):
                g = y[:, 0:128]
                return g * y[:, 128:256] * (1.0 + jnp.tanh(g))
            if part == 0:
                st["z4"] = _dot(paced(x(2)), w(1, 2))
                st["z3"] = _dot(_bf(x(5)), w(4, 5))
            elif part == 1:
                st["m4"] = short(0, st["z4"])
            elif part == 2:
                st["m2"] = long(0, 16, 17, 18, 19)
                st["h12"] = act(st["m4"] + st["m2"])
            elif part == 3:
                st["m3"] = short(1, st["z3"])
            elif part == 4:
                m5 = long(1, 20, 21, 22, 23)
                st["h21"] = act(st["m3"] + m5)
                st["m4"] = st["m4"] - m5
                st["m3"] = st["m3"] - st["m2"]
            elif part == 5:
                z = x(8)
                st["z1"] = _cat([_dot(paced(z[0:16]), w(7, 8)), _dot(_bf(z[16:32]), w(7, 8))], 0)
            elif part == 6:
                st["m1"] = short(2, st["z1"])
            elif part == 7:
                h11 = st["h11"] = act(st["m1"] + st["m4"] + long(2, 9, 10, 11, 12))
                h_s.at[u][:, 0:384] = _pk(_cat([h11, st["h21"] - h11, h11 + st["h12"]], 1))
            else:
                h22 = act(st["m1"] + st["m3"] + long(3, 13, 14, 15, 12))
                h_s.at[u][:, 384:896] = _pk(_cat([st["h11"] + h22, st["h12"] - h22, h22, st["h21"] + h22], 1))

        def ffn_down(lo, hi):
            first = True
            mark = _u32(st["acc"][1, 1])
            while lo < hi:
                n, k0 = divmod(lo, NU)
                k1 = min(NU, k0 + hi - lo)
                col = _tile((0, 1, 4, 5, 3, 6, 2)[n])
                a = _cat([wd_s[k, :, col] for k in range(k0, k1)], 1)
                b = _bf(_cat([h_s[k, :, col] for k in range(k0, k1)], 1))
                if hi == 1:
                    y = _cat([_dot_nt(paced(a[0:32]), b), _dot_nt(_bf(a[32:64]), b),
                              _dot_nt(_bf(a[64:96]), b), _dot_nt(_bf(a[80:112]), b)[32:64]], 0)
                elif first:
                    y = _dot_nt(paced(a), b)
                else:
                    head = [_after(never, mark, a[0:8, _tile(j)]) for j in range(k1 - k0)]
                    y = _dot_nt(_bf(_cat([_cat(head, 1), a[8:]], 0)), b)
                y = st["y"] = y if k0 == 0 else m_s[n] + y
                lo += k1 - k0
                first = False
                if k1 < NU or n < 5:
                    m_s[n] = y
                if k1 == NU and n == 1:
                    y_s[it, D // 2:, :128] = m_s[0] + y
                if k1 == NU and n == 3:
                    y_s[it, :D // 2, 128:] = m_s[2] + y
                if k1 == NU and n == 5:
                    y_s[it, :D // 2, :128] = m_s[4] + m_s[1] - m_s[3] + y
                if k1 == NU and n == 6:
                    y_s[it, D // 2:, 128:] = m_s[4] - m_s[0] + m_s[2] + y

        nv = -(-KV // CK)
        order = list(range(NC - 1, nv - 1, -1)) + list(range(nv))
        seq = [(i, c) for i in range(NI) for c in order]
        ffn = []
        for u in range(NU):
            ups = [(functools.partial(ffn_up, u, part), n, ops) for part, (n, ops) in
                   enumerate(((4, 4), (4, 12), (8, 20), (4, 12), (8, 28), (2, 4), (4, 12), (8, 31), (8, 34)))]
            ffn += [ups[0:3], ups[3:7], ups[7:9]]
        ffn += [[(functools.partial(ffn_down, 0, 1), 4, 9), (functools.partial(ffn_down, 1, 5), 14, 9)]]
        ffn += [[(functools.partial(ffn_down, lo, lo + 4), 14, 9)] for lo in range(5, 49, 4)]
        tape = []
        nf = 0
        for t in range(len(seq) + LAG):
            if t < len(seq):
                i, c = seq[t]
                lo, hi = max(c * CK, KV), (c + 1) * CK
                if hi > lo:
                    tape.append((functools.partial(qk, i, lo, hi), (hi - lo) // 16, 13))
            while nf < len(ffn) and (nf - 1 if nf + 1 < len(ffn) else nf + 1) * len(seq) <= (t + 1) * len(ffn):
                tape += ffn[nf]
                nf += 1
            if t >= LAG:
                i, c = seq[t - LAG]
                last = c == order[-1]
                tape.append((functools.partial(pv, i, c * CK, (c + 1) * CK, last), 2, 40 if last else 9))
        busy = [0] * 10 + [ops for _, n, ops in tape for _ in range(n)]
        nslot = len(busy) - 10
        share = [61 - busy[t] if 1 <= t < nslot - 4 else 0 for t in range(nslot)]
        cost = [0]
        for i, r, c0, d in work:
            cost.append(cost[-1] + 8 + 2.2 * (i % NQ == 0 and c0 == 0) + 4 * (r == 0)
                        + 3.5 * (i == 0 and r < 3) + 2 * (d == DH - 1))
        target, run, total = [], 0, sum(share)
        for w in share:
            run += w
            target.append(min(len(work), bisect.bisect_left(cost, cost[-1] * run / total)))
        for step, _, _ in tape:
            step()
        assert st["slot"] == nslot and st["spread"] == len(spread) and st["done"] == len(work)
        mark = _u32(st["y"][D // 2 - 8:])
        for r in range(S // 2 - 8, KV // 2 - 8, -8):
            kc_s[r:r + 8] = _after(never, mark, k_s[nxt, r:r + 8])
        return carry

    lax.fori_loop(0, NIT, trip, 0)

    @pl.when(jnp.max(bad_s[...]) > 0.0)
    def _():
        def guarded(n, carry):
            h, c = n // NQ, n % NQ
            r = lax.broadcasted_iota(jnp.int32, (32, BQ), 0) - DH // 2 * (h % 2)
            q = jnp.where((r >= 0) & (r < DH // 2), q_s[h // 2, c], jnp.uint32(0))
            s = _dot(_bf(k_s[h // 2]), _bf(_cat([q, jnp.zeros_like(q)], 0)))
            p = jnp.exp2(s - jnp.max(s, axis=0, keepdims=True))
            o_s[h, c] = _dot(_bf(v_s[h]), p.astype(_BF))
            return carry
        lax.fori_loop(0, H * NQ, guarded, 0)

    def attended(c, t):
        rows = []
        for p in range(NIT):
            e, o = o_s[2 * p, c, :, _tile(t)], o_s[2 * p + 1, c, :, _tile(t)]
            inv = 1.0 / jnp.where(row8 < 4, o[0:8], e[24:32])
            e, o = e * inv[4:5], o * inv[0:1]
            rows += [e[0:24], jnp.where(row8 < 4, e[24:32], o[0:8]), o[8:32]]
        return _cat(rows, 0)

    out_cp = []
    left = lax.broadcasted_iota(jnp.int32, (D, 128), 1) < 64
    for c in range(NQ):
        o = [attended(c, t) for t in range(4)]
        ot = [_cat(op, 0).astype(_BF) for op in _token_operands(lambda t, j: o[t][_tile(j, 64)])]
        y = _project(wt_s.at[3], lambda j: ot[j], (0, D // 2))
        ffn = [None] * 4
        for t in range(2):
            y0, y1 = y_s[2 * c, :, _tile(t)], y_s[2 * c + 1, :, _tile(t)]
            swapped = pltpu.roll(jnp.where(left, y1, y0), 64, 1)
            ffn[t], ffn[2 + t] = jnp.where(left, y0, swapped), jnp.where(left, swapped, y1)
        out = (2.0 * (y + _cat(ffn, 1)) + x_v[c].astype(_F32)).astype(_BF)
        if c + 1 < NQ:
            out_v[c] = out
            out_cp.append(pltpu.make_async_copy(out_v.at[c], out_hbm.at[:, pl.ds(c * BQ, BQ)], sems.at[5]))
            out_cp[-1].start()
        else:
            for j, (r, t) in enumerate(((0, 1), (0, 3), (1, 0), (1, 2), (0, 0), (0, 2), (1, 1), (1, 3))):
                last_v[j] = out[_tile(r, D // 2), _tile(t)]
                dst = out_hbm.at[pl.ds(r * D // 2, D // 2), pl.ds(c * BQ + 128 * t, 128)]
                out_cp.append(pltpu.make_async_copy(last_v.at[j], dst, sems.at[5]))
                out_cp[-1].start()
    for cp in out_cp:
        cp.wait()


@jax.jit
def pallas_parallel_sum__softmax_full_mha__glu_gated_swiglu__prompt_kernel(
    A_x: jax.Array,
    A_wqkv: jax.Array,
    A_wo: jax.Array,
    B_x: jax.Array,
    B_w1: jax.Array,
    B_w3: jax.Array,
    B_w2: jax.Array,
):
    del B_x
    any_spec = pl.BlockSpec(memory_space=pl.ANY)
    out = pl.pallas_call(
        _kernel,
        out_shape=jax.ShapeDtypeStruct((D, S), _BF),
        in_specs=[any_spec] * 6,
        out_specs=any_spec,
        scratch_shapes=[
            pltpu.VMEM((NQ, D, BQ), _BF),
            pltpu.VMEM((D, D), _BF),
            pltpu.VMEM((D, 2 * D), _BF),
            pltpu.VMEM((D, D), _BF),
            pltpu.VMEM((D, F), _BF),
            pltpu.VMEM((D, F), _BF),
            pltpu.VMEM((D, F), _BF),
            pltpu.VMEM((NQ - 1, D, BQ), _BF),
            pltpu.VMEM((8, D // 2, 128), _BF),
            pltpu.VMEM((4, D // 4, 17 * 128), _U32),
            pltpu.VMEM((NU, 12 * 64, 256), _U32),
            pltpu.VMEM((NU, D // 4, 7 * 128), _U32),
            pltpu.VMEM((NQ, 64, NX * 128), _U32),
            pltpu.VMEM((NIT, 32, NX * 128), _U32),
            pltpu.VMEM((NIT, S // 2, 128), _U32),
            pltpu.VMEM((NIT, NQ, 32, BQ), _U32),
            pltpu.VMEM((H, 16, S), _U32),
            pltpu.VMEM((NIT, 32, BQ), _U32),
            pltpu.VMEM((NIT, KV, 128), _U32),
            pltpu.VMEM((H, NQ, 32, BQ), _F32),
            pltpu.VMEM((NIT, D, 256), _F32),
            pltpu.VMEM((8, BQ), _F32),
            pltpu.VMEM((S // 2, 128), _U32),
            pltpu.VMEM((16, S), _U32),
            pltpu.VMEM((32, NX * 128), _U32),
            pltpu.VMEM((KV, 128), _U32),
            pltpu.VMEM((NQ, 2 * DH, BQ), _F32),
            pltpu.VMEM((NI, 24, BQ), _U32),
            pltpu.VMEM((2, KV // 16, DH // 2, 2, 1, 8, 128), _U32),
            pltpu.VMEM((2, KV // 16, DH, 2, 1, 8, 128), _F32),
            pltpu.VMEM((2, 2, DH + 2, 1, 2, 8, 128), _F32),
            pltpu.VMEM((S // 2, BQ), _U32),
            pltpu.VMEM((NI, KV // 2, BQ), _U32),
            pltpu.VMEM((NU, 64, 7 * 128), _U32),
            pltpu.VMEM((7, D // 2, 128), _F32),
            pltpu.SemaphoreType.DMA((6,)),
        ],
        compiler_params=pltpu.CompilerParams(vmem_limit_bytes=100 << 20),
    )(A_x.reshape(S, D).T, A_wqkv, A_wo, B_w1, B_w3, B_w2.T)
    return out.T.reshape(1, S, D)
```
